```python
import jax
import jax.numpy as jnp

def _softmax(x, axis=-1):
    return jax.nn.softmax(x, axis=axis)
def _gelu(x):
    return jax.nn.gelu(x, approximate=True)
def _silu(x):
    return jax.nn.silu(x)
def _sigmoid(x):
    return jax.nn.sigmoid(x)
def _layernorm(x, axis=-1, eps=1e-5):
    m = jnp.mean(x, axis=axis, keepdims=True)
    v = jnp.var(x, axis=axis, keepdims=True)
    return (x - m) / jnp.sqrt(v + eps)
def _scatter_add(tgt, idx, src, axis=0):
    return tgt.at[idx].add(src)
def _segment_sum(src, seg, n):
    return jax.ops.segment_sum(src, seg, n)
class _Rng:
    def __init__(self, key):
        self._k = key
    def _next(self):
        self._k, sub = jax.random.split(self._k)
        return sub
    def normal(self, shape):
        return jax.random.normal(self._next(), shape, dtype=jnp.bfloat16)
    def randint(self, lo, hi, shape):
        return jax.random.randint(self._next(), shape, lo, hi, dtype=jnp.int32)
    def uniform(self, shape, lo=0.0, hi=1.0):
        return jax.random.uniform(self._next(), shape, jnp.bfloat16, lo, hi)
    def permutation(self, n):
        return jax.random.permutation(self._next(), n)


kernel_name = 'parallel_sum__sliding_block_cached__glu_gated_swiglu__decode'

def setup_inputs():
    _rng = _Rng(jax.random.key(int.from_bytes(__import__("os").urandom(4), "little")))
    _w = (lambda a: (lambda t: t.astype(jnp.bfloat16) if jnp.issubdtype(t.dtype, jnp.floating) else t)(jnp.asarray(a)))
    def _A_setup():
        B, Sq, D = 4, 1, 640
        Hq, Hkv, Sk, Dh = 32, 32, 8192, 192
        assert Hq % Hkv == 0, (Hq, Hkv)
        return {
            "x": _w((lambda *s: _rng.normal(s) * 0.05)(B, Sq, D)),
            "k_cache": _w((lambda *s: _rng.normal(s) * 0.05)(B, Hkv, Sk, Dh)),
            "v_cache": _w((lambda *s: _rng.normal(s) * 0.05)(B, Hkv, Sk, Dh)),
            "wq": _w((lambda *s: _rng.normal(s) * 0.05)(D, Hq * Dh) * (D ** -0.5)),
            "wo": _w((lambda *s: _rng.normal(s) * 0.05)(Hq * Dh, D) * ((Hq * Dh) ** -0.5)),
        }
    _A_in = _A_setup()

    def _B_setup():
        B, S, D, F = 4, 1, 640, 1536
        return {
            "x": _w((lambda *s: _rng.normal(s) * 0.05)(B, S, D)),
            "w1": _w((lambda *s: _rng.normal(s) * 0.05)(D, F) * (2.0 / D) ** 0.5),
            "w3": _w((lambda *s: _rng.normal(s) * 0.05)(D, F) * (2.0 / D) ** 0.5),
            "w2": _w((lambda *s: _rng.normal(s) * 0.05)(F, D) * (2.0 / F) ** 0.5),
        }
    _B_in = _B_setup()

    return {
        "A_x": _A_in["x"],
        "A_k_cache": _A_in["k_cache"],
        "A_v_cache": _A_in["v_cache"],
        "A_wq": _A_in["wq"],
        "A_wo": _A_in["wo"],
        "B_x": _B_in["x"],
        "B_w1": _B_in["w1"],
        "B_w3": _B_in["w3"],
        "B_w2": _B_in["w2"],
    }

def reference(A_x, A_k_cache, A_v_cache, A_wq, A_wo, B_x, B_w1, B_w3, B_w2):
    def _A_ref(x, k_cache, v_cache, wq, wo):
        B, Sq, D = x.shape
        Hq, Dh = 32, 192
        Hkv, Sk = k_cache.shape[1], k_cache.shape[2]
        W = min(4096, max(256, Sk // 4))
        rep = Hq // Hkv
        q = (lambda x, *d: x.transpose(*d))((x @ wq).reshape(B, Sq, Hq, Dh), 0, 2, 1, 3)
        k = jnp.repeat(k_cache[:, :, Sk - W:, :], rep, axis=1)
        v = jnp.repeat(v_cache[:, :, Sk - W:, :], rep, axis=1)
        scores = jnp.einsum("bhqd,bhkd->bhqk", q, k) * (Dh ** -0.5)
        p = _softmax(scores, axis=-1)
        o = jnp.einsum("bhqk,bhkd->bhqd", p, v)
        return (lambda x, *d: x.transpose(*d))(o, 0, 2, 1, 3).reshape(B, Sq, Hq * Dh) @ wo

    def _B_ref(x, w1, w3, w2):
        gate = jnp.einsum("bsd,df->bsf", x, w1)
        up = jnp.einsum("bsd,df->bsf", x, w3)
        h = _silu(gate) * up
        out = jnp.einsum("bsf,fd->bsd", h, w2)
        return out

    x = A_x
    xn = _layernorm(x, axis=-1)
    return x + _A_ref(xn, A_k_cache, A_v_cache, A_wq, A_wo) + _B_ref(xn, B_w1, B_w3, B_w2)
```

```python
import functools

import jax
import jax.numpy as jnp
from jax import lax
import jax.experimental.pallas as pl
import jax.experimental.pallas.tpu as pltpu

_HQ, _DH = 32, 192
_G = 2
_R = _G * _DH
_NB = 6


def _kernel(x_hbm, kt_hbm, vt_hbm, wq_hbm, wo_hbm, w1_hbm, w3_hbm, w2_hbm, out_ref,
            x_v, wq_v, wo_v, w1_v, w3_v, w2_v, q_v, k_buf, v_buf, w_sem, k_sem, v_sem,
            *, nu, npair, sk, win):
    f32, bf16 = jnp.float32, jnp.bfloat16
    nb_, d = x_v.shape

    def k_copy(u, slot):
        return pltpu.make_async_copy(
            kt_hbm.at[pl.ds(u * _R, _R), pl.ds(sk - win, win)], k_buf.at[slot], k_sem.at[slot])

    def v_copy(u, slot):
        return pltpu.make_async_copy(
            vt_hbm.at[pl.ds(u * _R, _R), pl.ds(sk - win, win)], v_buf.at[slot], v_sem.at[slot])

    w_copies = [
        pltpu.make_async_copy(s, t, w_sem.at[i])
        for i, (s, t) in enumerate([(x_hbm, x_v), (wq_hbm, wq_v), (wo_hbm, wo_v),
                                    (w1_hbm, w1_v), (w3_hbm, w3_v), (w2_hbm, w2_v)])
    ]
    w_copies[0].start()
    w_copies[1].start()
    for i in range(_NB):
        k_copy(i, i).start()
        v_copy(i, i).start()
        if i == 0:
            w_copies[2].start()
    for c in w_copies[3:]:
        c.start()

    w_copies[0].wait()
    x = x_v[...].astype(f32)
    mu = jnp.mean(x, axis=-1, keepdims=True)
    xc = x - mu
    var = jnp.mean(xc * xc, axis=-1, keepdims=True)
    xn = xc / jnp.sqrt(var + 1e-5)
    xn8 = jnp.concatenate([xn, xn], axis=0).astype(bf16)

    w_copies[1].wait()
    for hp in range(npair):
        q_v[hp] = jnp.dot(xn8, wq_v[:, hp * _R:(hp + 1) * _R], preferred_element_type=f32)

    w_copies[2].wait()
    row = lax.broadcasted_iota(jnp.int32, (2 * nb_, _R), 0)
    col = lax.broadcasted_iota(jnp.int32, (2 * nb_, _R), 1)
    own = row - jnp.where(col >= _DH, nb_, 0)
    scale = _DH ** -0.5

    def body(u, acc):
        slot = lax.rem(u, _NB)
        b = u // npair
        hp = lax.rem(u, npair)
        mask = own == b
        q = jnp.where(mask, q_v[hp], 0.0).astype(bf16)
        k_copy(u, slot).wait()
        s = jnp.dot(q, k_buf[slot], preferred_element_type=f32) * scale

        @pl.when(u + _NB < nu)
        def _():
            k_copy(u + _NB, slot).start()

        m = jnp.max(s, axis=-1, keepdims=True)
        p = jnp.exp(s - m)
        l = jnp.sum(p, axis=-1, keepdims=True)
        v_copy(u, slot).wait()
        o = lax.dot_general(p.astype(bf16), v_buf[slot], (((1,), (1,)), ((), ())),
                            preferred_element_type=f32)

        @pl.when(u + _NB < nu)
        def _():
            v_copy(u + _NB, slot).start()

        o = jnp.where(mask, o / l, 0.0).astype(bf16)
        wo_blk = wo_v[pl.ds(pl.multiple_of(hp * _R, _R), _R), :]
        return acc + jnp.dot(o, wo_blk, preferred_element_type=f32)

    def ffn():
        w_copies[3].wait()
        gate = jnp.dot(xn8, w1_v[...], preferred_element_type=f32)
        w_copies[4].wait()
        up = jnp.dot(xn8, w3_v[...], preferred_element_type=f32)
        h = (gate * jax.nn.sigmoid(gate) * up).astype(bf16)
        w_copies[5].wait()
        return jnp.dot(h, w2_v[...], preferred_element_type=f32)[:nb_]

    acc = lax.fori_loop(0, nu // 2, body, jnp.zeros((2 * nb_, d), f32))
    res = x + ffn()
    acc = lax.fori_loop(nu // 2, nu, body, acc)
    out_ref[...] = (res + acc[:nb_] + acc[nb_:]).astype(out_ref.dtype)


@jax.jit
def pallas_parallel_sum__sliding_block_cached__glu_gated_swiglu__decode_kernel(
    A_x: jax.Array,
    A_k_cache: jax.Array,
    A_v_cache: jax.Array,
    A_wq: jax.Array,
    A_wo: jax.Array,
    B_x: jax.Array,
    B_w1: jax.Array,
    B_w3: jax.Array,
    B_w2: jax.Array,
):
    del B_x
    B, Sq, D = A_x.shape
    _, Hkv, Sk, Dh = A_k_cache.shape
    assert Sq == 1 and Hkv == _HQ and Dh == _DH
    win = min(4096, max(256, Sk // 4))
    F = B_w1.shape[1]
    npair = _HQ // _G
    nu = B * npair
    bf16 = jnp.bfloat16

    x2 = A_x.reshape(B, D)
    kt = jnp.swapaxes(A_k_cache, 2, 3).reshape(B * Hkv * Dh, Sk)
    vt = jnp.swapaxes(A_v_cache, 2, 3).reshape(B * Hkv * Dh, Sk)

    any_spec = pl.BlockSpec(memory_space=pl.ANY)
    out = pl.pallas_call(
        functools.partial(_kernel, nu=nu, npair=npair, sk=Sk, win=win),
        in_specs=[any_spec] * 8,
        out_specs=pl.BlockSpec(memory_space=pltpu.VMEM),
        out_shape=jax.ShapeDtypeStruct((B, D), A_x.dtype),
        scratch_shapes=[
            pltpu.VMEM((B, D), A_x.dtype),
            pltpu.VMEM((D, _HQ * Dh), bf16),
            pltpu.VMEM((_HQ * Dh, D), bf16),
            pltpu.VMEM((D, F), bf16),
            pltpu.VMEM((D, F), bf16),
            pltpu.VMEM((F, D), bf16),
            pltpu.VMEM((npair, 2 * B, _R), jnp.float32),
            pltpu.VMEM((_NB, _R, win), bf16),
            pltpu.VMEM((_NB, _R, win), bf16),
            pltpu.SemaphoreType.DMA((6,)),
            pltpu.SemaphoreType.DMA((_NB,)),
            pltpu.SemaphoreType.DMA((_NB,)),
        ],
        compiler_params=pltpu.CompilerParams(vmem_limit_bytes=100 * 1024 * 1024),
    )(x2, kt, vt, A_wq, A_wo, B_w1, B_w3, B_w2)
    return out.reshape(B, Sq, D)
```

```python
import functools

import jax
import jax.numpy as jnp
from jax import lax
import jax.experimental.pallas as pl
import jax.experimental.pallas.tpu as pltpu

_HQ, _DH = 32, 192
_G = 2
_R = _G * _DH
_T = 128


def _kernel(x_hbm, kt_hbm, vt_hbm, wq_hbm, wo_hbm, w1_hbm, w3_hbm, w2_hbm, out_ref,
            x_v, wq_v, wo_v, w1_v, w3_v, w2_v, q_v, p_v, k_buf, v_buf, w_sem, k_sem, v_sem,
            *, nu, npair, sk, win):
    f32, bf16 = jnp.float32, jnp.bfloat16
    nb_, d = x_v.shape

    ni, nj = _R // _T, win // _T

    def tile_copy(src, buf, sem, u, slot, i, j):
        return pltpu.make_async_copy(
            src.at[pl.ds(u * _R + i * _T, _T), pl.ds(sk - win + j * _T, _T)],
            buf.at[slot, pl.ds(i * _T, _T), pl.ds(j * _T, _T)], sem.at[j * ni + i])

    k_copy = functools.partial(tile_copy, kt_hbm, k_buf, k_sem)
    v_copy = functools.partial(tile_copy, vt_hbm, v_buf, v_sem)

    w_copies = [
        pltpu.make_async_copy(s, t, w_sem.at[i])
        for i, (s, t) in enumerate([(x_hbm, x_v), (wq_hbm, wq_v), (wo_hbm, wo_v),
                                    (w1_hbm, w1_v), (w3_hbm, w3_v), (w2_hbm, w2_v)])
    ]
    w_copies[0].start()
    w_copies[1].start()
    w_copies[2].start(priority=1)
    for j in range(nj):
        for i in range(ni):
            k_copy(0, 0, i, j).start()
    for c in w_copies[3:]:
        c.start(priority=1)

    w_copies[0].wait()
    x = x_v[...].astype(f32)
    mu = jnp.mean(x, axis=-1, keepdims=True)
    xc = x - mu
    var = jnp.mean(xc * xc, axis=-1, keepdims=True)
    xn = xc / jnp.sqrt(var + 1e-5)
    xn8 = jnp.concatenate([xn, xn], axis=0).astype(bf16)

    w_copies[1].wait()
    for hp in range(npair):
        q_v[hp] = jnp.dot(xn8, wq_v[:, hp * _R:(hp + 1) * _R], preferred_element_type=f32)

    row = lax.broadcasted_iota(jnp.int32, (2 * nb_, _R), 0)
    col = lax.broadcasted_iota(jnp.int32, (2 * nb_, _R), 1)
    own = row - jnp.where(col >= _DH, nb_, 0)
    scale = _DH ** -0.5

    def step(u, carry, do_pv=True, do_qk=True, more_k=True):
        acc, l_prev = carry
        slot = lax.rem(u, 2)
        if do_qk:
            q = jnp.where(own == u // npair, q_v[lax.rem(u, npair)], 0.0).astype(bf16)
        s, o = [], [0.0] * ni
        for j in range(nj):
            cs = slice(j * _T, (j + 1) * _T)
            for i in range(ni):
                if do_qk:
                    k_copy(u, slot, i, j).wait()
                    if more_k:
                        k_copy(u + 1, 1 - slot, i, j).start()
                if do_pv:
                    v_copy(u - 1, 1 - slot, i, j).wait()
                if do_qk:
                    v_copy(u, slot, i, j).start(priority=1)
            if do_qk:
                s.append(jnp.dot(q, k_buf[slot, :, cs], preferred_element_type=f32))
            if do_pv:
                p = p_v[:, cs].astype(bf16)
                for i in range(ni):
                    o[i] += lax.dot_general(p, v_buf[1 - slot, i * _T:(i + 1) * _T, cs],
                                            (((1,), (1,)), ((), ())), preferred_element_type=f32)
        if do_pv:
            o = jnp.concatenate(o, axis=1) / l_prev
            o = jnp.where(own == (u - 1) // npair, o, 0.0).astype(bf16)
            wo_blk = wo_v[pl.ds(pl.multiple_of(lax.rem(u - 1, npair) * _R, _R), _R), :]
            acc = acc + jnp.dot(o, wo_blk, preferred_element_type=f32)
        if do_qk:
            s = jnp.concatenate(s, axis=1) * scale
            e = jnp.exp(s - jnp.max(s, axis=-1, keepdims=True))
            l_prev = jnp.sum(e, axis=-1, keepdims=True)
            p_v[...] = e
        return acc, l_prev

    def ffn():
        w_copies[3].wait()
        gate = jnp.dot(xn8, w1_v[...], preferred_element_type=f32)
        w_copies[4].wait()
        up = jnp.dot(xn8, w3_v[...], preferred_element_type=f32)
        h = (gate * jax.nn.sigmoid(gate) * up).astype(bf16)
        w_copies[5].wait()
        return jnp.dot(h, w2_v[...], preferred_element_type=f32)[:nb_]

    carry = step(0, (jnp.zeros((2 * nb_, d), f32), None), do_pv=False)
    w_copies[2].wait()
    carry = lax.fori_loop(1, nu // 2, step, carry)
    res = x + ffn()
    carry = lax.fori_loop(nu // 2, nu - 1, step, carry)
    carry = step(nu - 1, carry, more_k=False)
    acc, _ = step(nu, carry, do_qk=False)
    out_ref[...] = (res + acc[:nb_] + acc[nb_:]).astype(out_ref.dtype)


@jax.jit
def pallas_parallel_sum__sliding_block_cached__glu_gated_swiglu__decode_kernel(
    A_x: jax.Array,
    A_k_cache: jax.Array,
    A_v_cache: jax.Array,
    A_wq: jax.Array,
    A_wo: jax.Array,
    B_x: jax.Array,
    B_w1: jax.Array,
    B_w3: jax.Array,
    B_w2: jax.Array,
):
    del B_x
    B, Sq, D = A_x.shape
    _, Hkv, Sk, Dh = A_k_cache.shape
    assert Sq == 1 and Hkv == _HQ and Dh == _DH
    win = min(4096, max(256, Sk // 4))
    F = B_w1.shape[1]
    npair = _HQ // _G
    nu = B * npair
    bf16 = jnp.bfloat16

    x2 = A_x.reshape(B, D)
    kt = jnp.swapaxes(A_k_cache, 2, 3).reshape(B * Hkv * Dh, Sk)
    vt = jnp.swapaxes(A_v_cache, 2, 3).reshape(B * Hkv * Dh, Sk)

    any_spec = pl.BlockSpec(memory_space=pl.ANY)
    out = pl.pallas_call(
        functools.partial(_kernel, nu=nu, npair=npair, sk=Sk, win=win),
        in_specs=[any_spec] * 8,
        out_specs=pl.BlockSpec(memory_space=pltpu.VMEM),
        out_shape=jax.ShapeDtypeStruct((B, D), A_x.dtype),
        scratch_shapes=[
            pltpu.VMEM((B, D), A_x.dtype),
            pltpu.VMEM((D, _HQ * Dh), bf16),
            pltpu.VMEM((_HQ * Dh, D), bf16),
            pltpu.VMEM((D, F), bf16),
            pltpu.VMEM((D, F), bf16),
            pltpu.VMEM((F, D), bf16),
            pltpu.VMEM((npair, 2 * B, _R), jnp.float32),
            pltpu.VMEM((2 * B, win), jnp.float32),
            pltpu.VMEM((2, _R, win), bf16),
            pltpu.VMEM((2, _R, win), bf16),
            pltpu.SemaphoreType.DMA((6,)),
            pltpu.SemaphoreType.DMA((_R * win // _T ** 2,)),
            pltpu.SemaphoreType.DMA((_R * win // _T ** 2,)),
        ],
        compiler_params=pltpu.CompilerParams(vmem_limit_bytes=100 * 1024 * 1024),
    )(x2, kt, vt, A_wq, A_wo, B_w1, B_w3, B_w2)
    return out.reshape(B, Sq, D)
```
